```python
import jax
import jax.numpy as jnp

def _softmax(x, axis=-1):
    return jax.nn.softmax(x, axis=axis)
def _gelu(x):
    return jax.nn.gelu(x, approximate=True)
def _silu(x):
    return jax.nn.silu(x)
def _sigmoid(x):
    return jax.nn.sigmoid(x)
def _layernorm(x, axis=-1, eps=1e-5):
    m = jnp.mean(x, axis=axis, keepdims=True)
    v = jnp.var(x, axis=axis, keepdims=True)
    return (x - m) / jnp.sqrt(v + eps)
def _scatter_add(tgt, idx, src, axis=0):
    return tgt.at[idx].add(src)
def _segment_sum(src, seg, n):
    return jax.ops.segment_sum(src, seg, n)
class _Rng:
    def __init__(self, key):
        self._k = key
    def _next(self):
        self._k, sub = jax.random.split(self._k)
        return sub
    def normal(self, shape):
        return jax.random.normal(self._next(), shape, dtype=jnp.bfloat16)
    def randint(self, lo, hi, shape):
        return jax.random.randint(self._next(), shape, lo, hi, dtype=jnp.int32)
    def uniform(self, shape, lo=0.0, hi=1.0):
        return jax.random.uniform(self._next(), shape, jnp.bfloat16, lo, hi)
    def permutation(self, n):
        return jax.random.permutation(self._next(), n)


kernel_name = 'standalone__modern_conv_block_slak__vision'

def setup_inputs():
    _rng = _Rng(jax.random.key(int.from_bytes(__import__("os").urandom(4), "little")))
    _w = (lambda a: (lambda t: t.astype(jnp.bfloat16) if jnp.issubdtype(t.dtype, jnp.floating) else t)(jnp.asarray(a)))
    H = W = 384
    C = 384
    K = 1
    return {
        "x": _w((lambda *s: _rng.normal(s) * 0.05)(1, H, W, C)),
        "dw": _w((lambda *s: _rng.normal(s) * 0.05)(K, K, C)),
        "w1": _w((lambda *s: _rng.normal(s) * 0.05)(C, 4 * C)),
        "w2": _w((lambda *s: _rng.normal(s) * 0.05)(4 * C, C)),
        "grn_g": _w((lambda *s: _rng.normal(s) * 0.05)(4 * C)),
        "grn_b": _w((lambda *s: _rng.normal(s) * 0.05)(4 * C)),
    }

def reference(x, dw, w1, w2, grn_g, grn_b):
    B, H, W, C = x.shape
    K = dw.shape[0]
    pad = K // 2
    xp = jnp.pad(x, ((0,0),(pad,pad),(pad,pad),(0,0)))
    out = jnp.zeros_like(x)
    for i in range(K):
        for j in range(K):
            out = out + xp[:, i:i+H, j:j+W, :] * dw[i, j][None, None, None, :]
    h = _layernorm(out, axis=-1)
    h = _gelu(h @ w1)
    gx = jnp.sqrt((h * h).sum(axis=(1, 2), keepdims=True) + 1e-6)
    nx = gx / (gx.mean(axis=-1, keepdims=True) + 1e-6)
    h = grn_g[None, None, None, :] * (h * nx) + grn_b[None, None, None, :] + h
    return x + h @ w2
```

```python
import functools
import math
import jax
import jax.numpy as jnp
import jax.experimental.pallas as pl
import jax.experimental.pallas.tpu as pltpu

TM = 1024
RC = 512
CACHE_EVERY = 4
NXB = 3
NHB = 3
NOB = 2
VMEM_LIMIT = 127 * 1024 * 1024

_C1 = math.sqrt(2.0 / math.pi)
_C2 = _C1 * 0.044715
_A = _C2 ** (1.0 / 3.0)
_KK = _C1 / _A
_HS = 0.5 / _A


def _body(x_hbm, dw_ref, w1_ref, w2_ref, g_ref, b_ref, o_hbm, h_hbm,
          xbuf, hbuf, obuf, w2s, ssq, xsem, hsem, osem, *, n, c, tm, rc, ce):
    nb = n // tm
    ncache = nb // ce
    f32 = jnp.float32

    def x_copy(i, slot):
        return pltpu.make_async_copy(x_hbm.at[pl.ds(pl.multiple_of(i * tm, tm), tm)], xbuf.at[slot], xsem.at[slot])

    def is_cached(i):
        return i % ce == ce - 1

    def hbm_idx(i):
        return i - i // ce

    def h_slot(i):
        return jnp.where(is_cached(i), NHB + i // ce, hbm_idx(i) % NHB)

    def h_out_copy(u):
        s = u % NHB
        return pltpu.make_async_copy(hbuf.at[s], h_hbm.at[pl.ds(pl.multiple_of(u * tm, tm), tm)], hsem.at[s])

    def h_in_copy(u):
        s = u % NHB
        return pltpu.make_async_copy(h_hbm.at[pl.ds(pl.multiple_of(u * tm, tm), tm)], hbuf.at[s], hsem.at[s])

    def o_copy(i, slot):
        return pltpu.make_async_copy(obuf.at[slot], o_hbm.at[pl.ds(pl.multiple_of(i * tm, tm), tm)], osem.at[slot])

    nu = nb - ncache
    for j in range(NXB - 1):
        x_copy(j, j).start()
    ssq[...] = jnp.zeros_like(ssq)
    dw = dw_ref[...].astype(f32)

    def phase1(i, carry):
        nxt = i + NXB - 1
        x_copy(nxt % nb, nxt % NXB).start()
        x_copy(i, i % NXB).wait()
        u = hbm_idx(i)

        @pl.when(jnp.logical_and(jnp.logical_not(is_cached(i)), u >= NHB))
        def _():
            h_out_copy(u - NHB).wait()

        xs = i % NXB
        hs = h_slot(i)
        for r in range(tm // rc):
            rows = pl.ds(r * rc, rc)
            o = xbuf[xs, rows, :].astype(f32) * dw
            m = jnp.mean(o, axis=-1, keepdims=True)
            d = o - m
            v = jnp.mean(d * d, axis=-1, keepdims=True)
            a = (d * (jax.lax.rsqrt(v + 1e-5) * _A)).astype(jnp.bfloat16)
            y = jnp.dot(a, w1_ref[...], preferred_element_type=f32)
            hh = y * (1.0 + jnp.tanh(y * (y * y + _KK)))
            hbuf[hs, rows, :] = hh.astype(jnp.bfloat16)
            ssq[...] += (hh * hh).reshape(rc // 8, 8, 4 * c).sum(axis=0)

        @pl.when(jnp.logical_not(is_cached(i)))
        def _():
            h_out_copy(u).start()
        return carry

    jax.lax.fori_loop(0, nb, phase1, 0)
    for u in range(nu - NHB, nu):
        h_out_copy(u).wait()
    for u in range(NHB - 1):
        h_in_copy(u).start()

    gx = jnp.sqrt(jnp.sum(ssq[...], axis=0, keepdims=True) * (_HS * _HS) + 1e-6)
    nx = gx / (jnp.mean(gx, axis=-1, keepdims=True) + 1e-6)
    s = (g_ref[...].astype(f32) * nx + 1.0) * _HS
    st = jnp.transpose(jnp.broadcast_to(s, (128, 4 * c)))
    for j in range(c // 128):
        cols = pl.ds(j * 128, 128)
        w2s[:, cols] = (w2_ref[:, cols].astype(f32) * st).astype(jnp.bfloat16)
    bias = jnp.dot(jnp.broadcast_to(b_ref[...], (16, 4 * c)), w2_ref[...], preferred_element_type=f32)[0:1]

    def phase2(i, carry):
        nxt = i + NXB - 1

        @pl.when(nxt < nb)
        def _():
            x_copy(nxt, (nb + nxt) % NXB).start()
        u = hbm_idx(i)

        @pl.when(jnp.logical_not(is_cached(i)))
        def _():
            @pl.when(u + NHB - 1 < nu)
            def _():
                h_in_copy(u + NHB - 1).start()
            h_in_copy(u).wait()

        xs = (nb + i) % NXB
        x_copy(i, xs).wait()
        os_ = i % NOB

        @pl.when(i >= NOB)
        def _():
            o_copy(i - NOB, os_).wait()

        hs = h_slot(i)
        for r in range(tm // rc):
            rows = pl.ds(r * rc, rc)
            y = jnp.dot(hbuf[hs, rows, :], w2s[...], preferred_element_type=f32)
            obuf[os_, rows, :] = (y + bias + xbuf[xs, rows, :].astype(f32)).astype(jnp.bfloat16)
        o_copy(i, os_).start()
        return carry

    jax.lax.fori_loop(0, nb, phase2, 0)
    for i in range(nb - NOB, nb):
        o_copy(i, i % NOB).wait()


@jax.jit
def pallas_standalone__modern_conv_block_slak__vision_kernel(x, dw, w1, w2, grn_g, grn_b):
    bsz, hh, ww, c = x.shape
    assert bsz == 1 and dw.shape[0] == 1 and dw.shape[1] == 1
    n = hh * ww
    tm, rc, ce = TM, RC, CACHE_EVERY
    nb = n // tm
    ncache = nb // ce
    vm = pl.BlockSpec(memory_space=pltpu.VMEM)
    hbm = pl.BlockSpec(memory_space=pl.ANY)
    out, _ = pl.pallas_call(
        functools.partial(_body, n=n, c=c, tm=tm, rc=rc, ce=ce),
        in_specs=[hbm, vm, vm, vm, vm, vm],
        out_specs=[hbm, hbm],
        out_shape=[jax.ShapeDtypeStruct((n, c), x.dtype),
                   jax.ShapeDtypeStruct(((nb - ncache) * tm, 4 * c), jnp.bfloat16)],
        scratch_shapes=[
            pltpu.VMEM((NXB, tm, c), x.dtype),
            pltpu.VMEM((NHB + ncache, tm, 4 * c), jnp.bfloat16),
            pltpu.VMEM((NOB, tm, c), x.dtype),
            pltpu.VMEM((4 * c, c), jnp.bfloat16),
            pltpu.VMEM((8, 4 * c), jnp.float32),
            pltpu.SemaphoreType.DMA((NXB,)),
            pltpu.SemaphoreType.DMA((NHB,)),
            pltpu.SemaphoreType.DMA((NOB,)),
        ],
        compiler_params=pltpu.CompilerParams(vmem_limit_bytes=VMEM_LIMIT),
    )(x.reshape(n, c), dw.reshape(1, c), w1, w2, grn_g.reshape(1, 4 * c), grn_b.reshape(1, 4 * c))
    return out.reshape(x.shape)
```

```python
import functools
import math
import jax
import jax.numpy as jnp
import jax.experimental.pallas as pl
import jax.experimental.pallas.tpu as pltpu

R = 256
U = 2
NCACHE = 58
NXB = 6
NHB = 6
NOB = 4
VMEM_LIMIT = 127 * 1024 * 1024
PH1 = True
PH2 = True
DMA = True
W11 = (0.1, 1.0)
W13 = (0.06, 1.0)
W21 = (0.02, 1.0)
W23 = (0.02, 1.0)
TIE1 = ()
TIE2 = (5, 9, 10)
TIE_H = False
LAG = 2
REL3 = ()
REL4 = ()
OPAQUE = True
RG = 16
REL1 = "mem"
GK = (0,)
G0 = True
W10 = (0.02, 1.0)
REL2 = (5,)
SPLIT = False
STEP1 = True
STEP2 = False
OPAQUE1 = False
OPAQUE2 = True
TIE3 = (0, 1, 2)
TIE1H = (0, 1)
TIE4 = (0, 1, 2, 3, 4, 5)
F_LP = {"XLA_TPU_FORCE_LP_LLO_SCHEDULER": True}
F_EV = {"XLA_TPU_EVENLY_DISTRIBUTE_CRITICAL_NODES": True}
FLAGS = F_EV

_C1 = math.sqrt(2.0 / math.pi)
_C2 = _C1 * 0.044715
_A = _C2 ** (1.0 / 3.0)
_KK = _C1 / _A
_HS = 0.5 / _A

_V = ((-1, 0, 0, 0, 1, 0, -1, 1, 1), (-1, 0, 0, 1, 0, -1, 0, 0, 0), (1, 0, 0, 1, 0, 0, 1, 0, 0),
      (0, 0, -1, 0, 0, 0, 0, 0, 0), (0, 0, 0, 0, 1, 0, 0, 0, 0), (0, 0, 0, 0, 0, 1, 0, 0, 0),
      (1, 0, 0, 0, 0, 0, 0, 0, 0), (1, 0, 0, 0, -1, 0, 0, 0, 0), (0, 0, -1, 0, 1, 0, 0, 1, 0),
      (1, 0, 0, 0, 0, 1, 1, 0, 0), (0, 0, 1, 0, 0, 1, 0, 0, 1), (-1, 0, 0, 0, 1, 0, 0, 1, 0),
      (0, 1, 1, 0, -1, 0, 0, 0, 0), (0, 1, 0, 0, 1, 0, 0, 1, 0), (1, 0, 0, 0, -1, 0, 1, 0, 0))


def _left_forms(a, unit, rest):
    a0, a1, a2, a3, a4, a5 = a
    t0 = a3 - a5
    t1 = a4 - a5
    t2 = a2 - t0
    t3 = a0 - t2
    t4 = a1 + t3
    t5 = t4 - t0
    t6 = a2 - t1
    t7 = a2 + a5
    t8 = t1 + t5
    t9 = t8 - a0
    return (unit(2), unit(1), unit(4), rest(t3), rest(t8), rest(t9), rest(t4), rest(t5),
            rest(t2), rest(t6), rest(t7), rest(t0), unit(0), unit(3), rest(t1))


def _combine(p):
    n7 = p[8] + p[11]
    n6 = p[7] - p[6]
    n5 = p[4] + n6
    n4 = p[0] - n7
    n3 = p[14] + n5
    n2 = p[9] + n4 + n3
    n1 = p[5] + n2
    return (n1 - n4 + p[1] + p[6], p[12] + n7 + p[3] - n6, n1 - p[3],
            p[2] - n3, p[13] + n5 - p[11], p[10] - n2)


def _interleave(main, *side):
    items = [((j + 1.0) / len(main), 1, j, f) for j, f in enumerate(main)]
    for st, begin, end in side:
        items += [(begin + (end - begin) * (j + 1.0) / len(st) - 1e-9, 0, j, f) for j, f in enumerate(st)]
    items.sort(key=lambda t: t[:3])
    pending = []
    for _, is_main, _, f in items:
        if is_main:
            f(pending)
            pending = []
        else:
            pending = pending + list(f())


def _body(x_hbm, dw_ref, w1_ref, w2_ref, g_ref, b_ref, o_hbm, h_hbm,
          xbuf, hbuf, ssq, zref, xsem, hsem, osem, *, n, c, rr, ncache):
    tm = 2 * rr
    nb = n // tm
    nu = nb - ncache
    f32, bf16, i32 = jnp.float32, jnp.bfloat16, jnp.int32
    hc = 4 * c
    kb, nbk = c // 3, hc // 3
    rw = rr // 2

    def pack(lo, hi):
        return pltpu.bitcast(pltpu.pack_elementwise([lo, hi], packed_dtype=bf16), i32)

    def unpack(w):
        return [pltpu.unpack_elementwise(w, index=k, packed_dtype=bf16, unpacked_dtype=f32) for k in range(2)]

    def x_copy(i, slot):
        return pltpu.make_async_copy(x_hbm.at[pl.ds(pl.multiple_of(i * tm, tm), tm)], xbuf.at[slot], xsem.at[slot])

    def cached_before(i):
        return (i * ncache) // nb

    def is_cached(i):
        return cached_before(i + 1) > cached_before(i)

    def hbm_idx(i):
        return i - cached_before(i)

    def h_slot(i):
        return jnp.where(is_cached(i), NHB + cached_before(i), hbm_idx(i) % NHB)

    def h_out_copy(u):
        s = u % NHB
        return pltpu.make_async_copy(hbuf.at[s], h_hbm.at[pl.ds(pl.multiple_of(u * rr, rr), rr)], hsem.at[s])

    def h_in_copy(u):
        s = u % NHB
        return pltpu.make_async_copy(h_hbm.at[pl.ds(pl.multiple_of(u * rr, rr), rr)], hbuf.at[s], hsem.at[s])

    def right_forms(blk, dst):
        for r in range(15):
            terms = sorted(((cf, j) for j, cf in enumerate(_V[r]) if cf), key=lambda t: -t[0])
            acc = blk(*divmod(terms[0][1], 3))
            if terms[0][0] < 0:
                acc = -acc
            for cf, j in terms[1:]:
                acc = acc + blk(*divmod(j, 3)) if cf > 0 else acc - blk(*divmod(j, 3))
            dst(r, acc.astype(bf16))

    def products(lhs, rhs, put, never):
        rows = {}

        def piece(r, t):
            def run(ties):
                v = lhs(r, t)
                if ties:
                    tie = functools.reduce(jnp.bitwise_or, [pltpu.bitcast(z, i32) for z in ties])
                    head = jnp.where(never, tie, v[:, :128])
                    v = head if v.shape[1] == 128 else jnp.concatenate([head, v[:, 128:]], axis=1)
                rows.setdefault(r, []).append(v)
                if t == rr // 16 - 1:
                    a = pltpu.bitcast(jnp.concatenate(rows.pop(r), axis=0), bf16)
                    res = jnp.dot(a, rhs(r), preferred_element_type=f32)
                    put(r, res)
                    last.setdefault("res", []).append(res)
                last["t"] = t
            return run
        return [piece(r, t) for r in range(15) for t in range(rr // 16)]

    last = {}

    def after_matmul(w, never):
        if len(last.get("res", ())) < LAG:
            return w
        t = (last["t"] // RG) * RG
        return jnp.where(never, pltpu.bitcast(last["res"][-LAG][16 * t:16 * t + 8, :128], w.dtype), w)

    def never_mask():
        last.clear()
        return (jax.lax.broadcasted_iota(i32, (8, 128), 0) + zref[0]) < 0

    def run_loop(pre, work, post, bufs, stepdma):
        def region(k, carry):
            if stepdma:
                for q in range(U):
                    if DMA:
                        pre(k * U + q)
                        work(k * U + q, never_mask(), *bufs[q % 2])
                        post(k * U + q)
                    else:
                        pl.when(k < 100000 + q)(lambda: work(k * U + q, never_mask(), *bufs[q % 2]))
                return carry
            if DMA:
                for q in range(U):
                    pre(k * U + q)
            never = never_mask()
            for q in range(U):
                if SPLIT:
                    pl.when(k < 100000)(functools.partial(work, k * U + q, never, *bufs[q % 2]))
                else:
                    work(k * U + q, never, *bufs[q % 2], q=q)
            if DMA:
                for q in range(U):
                    post(k * U + q)
            return carry
        jax.lax.fori_loop(0, nb // U, region, 0)

    zref[0] = 0
    zref[1] = 0

    opaque = [OPAQUE1]

    def wview(ref):
        return ref.at[zref[0] if opaque[0] else 0]

    def rview(ref):
        return ref.at[zref[1] if opaque[0] else 0]

    if DMA:
        for j in range(NXB):
            x_copy(j, j).start()
    ssq[...] = jnp.zeros_like(ssq)

    def pass1(w1c, fa, fb, pa, pb):
        w1c = w1c.bitcast(bf16)
        dw = dw_ref[...].astype(f32)

        def put(r, v):
            w1c[pl.ds(r * kb, kb), :] = v
        right_forms(lambda j, k: w1_ref[j * kb:(j + 1) * kb, k * nbk:(k + 1) * nbk].astype(f32), put)

        def layer_norm(xv):
            o = xv * dw
            m = jnp.sum(o, axis=-1, keepdims=True) * (1.0 / c)
            d = o - m
            v = jnp.sum(d * d, axis=-1, keepdims=True)
            return d * jax.lax.rsqrt(v * (1.0 / (c * _A * _A)) + 1e-5 / (_A * _A))

        def s1(xs, fs, never=None):
            f = wview(fs).bitcast(bf16)
            gate = None
            if never is not None and REL1 == "mem":
                wview(fs)[pl.ds(rw, 8), pl.ds(0, 128)] = jnp.zeros((8, 128), i32)
                gate = rview(fs)[pl.ds(rw, 8), pl.ds(0, 128)]

            def piece(t):
                def run():
                    a = []
                    for half in range(2):
                        w = pltpu.bitcast(xbuf[xs, pl.ds(half * rr + 16 * t, 16), :], i32)
                        if gate is not None:
                            w = jnp.concatenate([jnp.where(never, gate, w[:, 128 * k:128 * k + 128]) if k in GK
                                                 else w[:, 128 * k:128 * k + 128] for k in range(3)], axis=1)
                        elif never is not None and REL1:
                            w = jnp.concatenate([after_matmul(w[:, :128], never), w[:, 128:]], axis=1)
                        ln = layer_norm(jnp.concatenate(unpack(w), axis=0))
                        a += [ln[:, j * kb:(j + 1) * kb] for j in range(3)]
                    lf = _left_forms(a, lambda j: a[j], lambda v: v)
                    for r in range(15):
                        f[pl.ds(16 * t, 16), pl.ds(r * kb, kb)] = lf[r].astype(bf16)
                    return [lf[r][8 * k:8 * k + 8] for r in TIE1 for k in TIE1H]
                return run
            return [piece(t) for t in range(rr // 16)]

        def s2(fs, ps, never=None):
            fs, ps = rview(fs), wview(ps)

            def put(r, v):
                ps[:, pl.ds(r * nbk, nbk)] = v
            return products(lambda r, t: fs[pl.ds(8 * t, 8), pl.ds(r * kb, kb)],
                            lambda r: w1c[pl.ds(r * kb, kb), :], put, never)

        def s3(hs, ps, never):
            ps = rview(ps)
            acc = {}

            def piece(j, t):
                def run():
                    p = [ps[pl.ds(16 * t, 16), pl.ds(r * nbk + 128 * j, 128)] for r in range(15)]
                    for r in REL3:
                        p[r] = jnp.concatenate([after_matmul(p[r][:8], never), after_matmul(p[r][8:], never)], axis=0)
                    cs = _combine(p)
                    ties = []
                    for k in range(3):
                        cols = pl.ds(k * nbk + 128 * j, 128)
                        if t == 0:
                            acc[k] = ssq[:, cols]
                        for half in range(2):
                            y = cs[3 * half + k]
                            hh = y * (1.0 + jnp.tanh(y * (y * y + _KK)))
                            w = pack(hh[:8], hh[8:])
                            hbuf[hs, pl.ds(half * rw + 8 * t, 8), cols] = w
                            sq = hh * hh
                            acc[k] = acc[k] + (sq[:8] + sq[8:])
                            ties.append(w)
                        if t == rr // 16 - 1:
                            ssq[:, cols] = acc[k]
                    return [ties[k] for k in TIE3] if TIE_H else [acc[k] for k in TIE3]
                return run
            return [piece(j, t) for j in range(nbk // 128) for t in range(rr // 16)]

        if DMA:
            x_copy(0, 0).wait()
            x_copy(1, 1).wait()
        for f in s1(0, fa):
            f()
        _interleave(s2(fa, pa, never_mask()), (s1(1, fb), 0.1, 1.0))
        if DMA:
            for j in range(2):
                x_copy(NXB + j, j).start()

        def pre(i):
            x_copy((i + 2) % nb, (i + 2) % NXB).wait()
            u = hbm_idx(i)

            @pl.when(jnp.logical_and(jnp.logical_not(is_cached(i)), u >= NHB))
            def _():
                h_out_copy(u - NHB).wait()

        def work(i, never, f0, f1, p0, p1, q=0):
            _interleave(s2(f1, p1, never), (s1((i + 2) % NXB, f0, never if q else None),) + W11, (s3(h_slot(i), p0, never),) + (W13 if q else W10))

        def post(i):
            nxt = i + NXB + 2

            @pl.when(i < nb - 2)
            def _():
                x_copy(nxt % nb, nxt % NXB).start()

            @pl.when(jnp.logical_not(is_cached(i)))
            def _():
                h_out_copy(hbm_idx(i)).start()

        run_loop(pre, work, post, ((fa, fb, pa, pb), (fb, fa, pb, pa)), STEP1)

    if PH1:
        pl.run_scoped(pass1,
                      pltpu.VMEM((15 * kb // 2, nbk), i32),
                      pltpu.VMEM((1, rw + 8, 15 * kb), i32), pltpu.VMEM((1, rw + 8, 15 * kb), i32),
                      pltpu.VMEM((1, rr, 15 * nbk), f32), pltpu.VMEM((1, rr, 15 * nbk), f32))
    if DMA:
        for u in range(nu - NHB, nu):
            if PH1:
                h_out_copy(u).wait()
        for u in range(NHB):
            if PH2:
                h_in_copy(u).start()

    def pass2(w2c, fa, fb, pa, pb, obuf):
        w2c = w2c.bitcast(bf16)
        opaque[0] = OPAQUE2

        def o_copy(i, slot):
            return pltpu.make_async_copy(obuf.at[slot], o_hbm.at[pl.ds(pl.multiple_of(i * tm, tm), tm)], osem.at[slot])

        gx = jnp.sqrt(jnp.sum(ssq[...], axis=0, keepdims=True) * (_HS * _HS) + 1e-6)
        nx = gx / (jnp.mean(gx, axis=-1, keepdims=True) + 1e-6)
        s = (g_ref[...].astype(f32) * nx + 1.0) * _HS
        st = jnp.transpose(jnp.broadcast_to(s, (128, hc)))

        def put(r, v):
            w2c[:, pl.ds(r * kb, kb)] = v
        right_forms(lambda j, k: w2_ref[j * nbk:(j + 1) * nbk, k * kb:(k + 1) * kb].astype(f32)
                    * st[j * nbk:(j + 1) * nbk], put)
        bias = jnp.dot(jnp.broadcast_to(b_ref[...], (16, hc)), w2_ref[...], preferred_element_type=f32)
        slot_of = {}
        for r, v in enumerate(_left_forms([0] * 6, lambda j: j, lambda v: None)):
            slot_of[r] = ("unit", v) if v is not None else ("rest", sum(1 for q in slot_of.values() if q[0] == "rest"))

        def s1(hs, fs, never=None):
            fs = wview(fs)

            def piece(t, j):
                def run():
                    a = [hbuf[hs, pl.ds((q // 3) * rw + 8 * t, 8), pl.ds((q % 3) * nbk + 128 * j, 128)]
                         for q in range(6)]
                    if never is not None:
                        a = [after_matmul(v, never) if q in REL2 else v for q, v in enumerate(a)]
                    a = [unpack(v) for v in a]
                    lo, hi = [_left_forms([v[k] for v in a], lambda q: None, lambda v: v) for k in range(2)]
                    ties = []
                    for r in range(15):
                        if slot_of[r][0] == "rest":
                            w = pack(lo[r], hi[r])
                            fs[pl.ds(slot_of[r][1] * rw + 8 * t, 8), pl.ds(128 * j, 128)] = w
                            if r in TIE2:
                                ties.append(w)
                    return ties
                return run
            return [piece(t, j) for t in range(rr // 16) for j in range(nbk // 128)]

        def s2(hs, fs, ps, never=None):
            fs, ps = rview(fs), wview(ps)

            def lhs(r, t):
                kind, q = slot_of[r]
                if kind == "unit":
                    return hbuf[hs, pl.ds((q // 3) * rw + 8 * t, 8), pl.ds((q % 3) * nbk, nbk)]
                return fs[pl.ds(q * rw + 8 * t, 8), :]

            def put(r, v):
                ps[:, pl.ds(r * kb, kb)] = v
            return products(lhs, lambda r: w2c[:, pl.ds(r * kb, kb)], put, never)

        def s3(xs, os_, ps, never):
            ps = rview(ps)

            def piece(t):
                def run():
                    p = [ps[pl.ds(16 * t, 16), pl.ds(r * kb, kb)] for r in range(15)]
                    for r in REL4:
                        p[r] = jnp.concatenate([after_matmul(p[r][:8], never), after_matmul(p[r][8:], never)], axis=0)
                    cs = _combine(p)
                    ties = []
                    for q, y in enumerate(cs):
                        half, k = divmod(q, 3)
                        rows = pl.ds(half * rr + 16 * t, 16)
                        cols = pl.ds(k * kb, kb)
                        y = y + bias[:, k * kb:(k + 1) * kb] + xbuf[xs, rows, cols].astype(f32)
                        obuf[os_, rows, cols] = y.astype(bf16)
                        ties += [y[:8], y[8:]] if q in TIE4 else []
                    return ties
                return run
            return [piece(t) for t in range(rr // 16)]

        if DMA:
            h_in_copy(0).wait()
            h_in_copy(1).wait()
            if not PH1:
                x_copy(0, 0).wait()
                x_copy(1, 1).wait()
        for f in s1(0, fa):
            f()
        _interleave(s2(0, fa, pa, never_mask()), (s1(1, fb), 0.05, 1.0))
        if DMA:
            h_in_copy(NHB).start()

        def pre(i):
            @pl.when(jnp.logical_and(i + 2 < nb, jnp.logical_not(is_cached(i + 2))))
            def _():
                h_in_copy(hbm_idx(i + 2)).wait()

            @pl.when(i > 1)
            def _():
                x_copy(i, (nb + i) % NXB).wait()

            @pl.when(i >= NOB)
            def _():
                o_copy(i - NOB, i % NOB).wait()

        def work(i, never, f0, f1, p0, p1, q=0):
            j1 = jnp.minimum(i + 1, nb - 1)
            j2 = jnp.minimum(i + 2, nb - 1)
            _interleave(s2(h_slot(j1), f1, p1, never), (s1(h_slot(j2), f0, never if q or G0 else None),) + W21,
                        (s3((nb + i) % NXB, i % NOB, p0, never),) + W23)

        def post(i):
            o_copy(i, i % NOB).start()

            @pl.when(i + NXB < nb)
            def _():
                x_copy(i + NXB, (nb + i) % NXB).start()

            u = hbm_idx(i + 1)

            @pl.when(jnp.logical_and(jnp.logical_not(is_cached(i + 1)), u + NHB < nu))
            def _():
                h_in_copy(u + NHB).start()

        run_loop(pre, work, post, ((fa, fb, pa, pb), (fb, fa, pb, pa)), STEP2)
        if DMA:
            for i in range(nb - NOB, nb):
                o_copy(i, i % NOB).wait()
        else:
            o_copy(0, 0).start()
            o_copy(0, 0).wait()

    if PH2:
        pl.run_scoped(pass2,
                      pltpu.VMEM((nbk // 2, 15 * kb), i32),
                      pltpu.VMEM((1, 10 * rw, nbk), i32), pltpu.VMEM((1, 10 * rw, nbk), i32),
                      pltpu.VMEM((1, rr, 15 * kb), f32), pltpu.VMEM((1, rr, 15 * kb), f32),
                      pltpu.VMEM((NOB, tm, c), bf16))
    else:
        if DMA:
            for j in range(2, NXB):
                x_copy(j, (nb + j) % NXB).wait()
        h_out_copy(0).start()
        h_out_copy(0).wait()
        xbuf[0, 0:8, :] = ssq[:, 0:c].astype(bf16)
        cp = pltpu.make_async_copy(xbuf.at[0], o_hbm.at[pl.ds(0, tm)], osem.at[0])
        cp.start()
        cp.wait()


@jax.jit
def pallas_standalone__modern_conv_block_slak__vision_kernel(x, dw, w1, w2, grn_g, grn_b):
    bsz, hh, ww, c = x.shape
    assert bsz == 1 and dw.shape[0] == 1 and dw.shape[1] == 1
    n = hh * ww
    tm, ncache = 2 * R, NCACHE
    nb = n // tm
    vm = pl.BlockSpec(memory_space=pltpu.VMEM)
    hbm = pl.BlockSpec(memory_space=pl.ANY)
    out, _ = pl.pallas_call(
        functools.partial(_body, n=n, c=c, rr=R, ncache=ncache),
        in_specs=[hbm, vm, vm, vm, vm, vm],
        out_specs=[hbm, hbm],
        out_shape=[jax.ShapeDtypeStruct((n, c), x.dtype),
                   jax.ShapeDtypeStruct(((nb - ncache) * tm // 2, 4 * c), jnp.int32)],
        scratch_shapes=[
            pltpu.VMEM((NXB, tm, c), x.dtype),
            pltpu.VMEM((NHB + ncache, tm // 2, 4 * c), jnp.int32),
            pltpu.VMEM((8, 4 * c), jnp.float32),
            pltpu.SMEM((2,), jnp.int32),
            pltpu.SemaphoreType.DMA((NXB,)),
            pltpu.SemaphoreType.DMA((NHB,)),
            pltpu.SemaphoreType.DMA((NOB,)),
        ],
        compiler_params=pltpu.CompilerParams(vmem_limit_bytes=VMEM_LIMIT, flags=FLAGS),
    )(x.reshape(n, c), dw.reshape(1, c), w1, w2, grn_g.reshape(1, 4 * c), grn_b.reshape(1, 4 * c))
    return out.reshape(x.shape)
```

```python
import functools
import math

import jax
import jax.numpy as jnp
import jax.experimental.pallas as pl
import jax.experimental.pallas.tpu as pltpu

R = 256
NCACHE = 64
NHB = 6
NXB = 4
NX2 = 16
OB = 4
VMEM_LIMIT = 128 * 1024 * 1024
W11 = (0.1, 1.0)
W13 = (0.02, 1.0)
W21 = (0.01, 0.33)
TIE2 = (5, 9, 10)
ORDER2 = (0, 1, 2, 12, 13, 11, 8, 6, 7, 4, 14, 9, 3, 5, 10)
FLAGS = {"XLA_TPU_EVENLY_DISTRIBUTE_CRITICAL_NODES": True}
PH1 = True
PH2 = True

_C1 = math.sqrt(2.0 / math.pi)
_A = (_C1 * 0.044715) ** (1.0 / 3.0)
_KK = _C1 / _A
_HS = 0.5 / _A

_V = ((-1, 0, 0, 0, 1, 0, -1, 1, 1), (-1, 0, 0, 1, 0, -1, 0, 0, 0), (1, 0, 0, 1, 0, 0, 1, 0, 0),
      (0, 0, -1, 0, 0, 0, 0, 0, 0), (0, 0, 0, 0, 1, 0, 0, 0, 0), (0, 0, 0, 0, 0, 1, 0, 0, 0),
      (1, 0, 0, 0, 0, 0, 0, 0, 0), (1, 0, 0, 0, -1, 0, 0, 0, 0), (0, 0, -1, 0, 1, 0, 0, 1, 0),
      (1, 0, 0, 0, 0, 1, 1, 0, 0), (0, 0, 1, 0, 0, 1, 0, 0, 1), (-1, 0, 0, 0, 1, 0, 0, 1, 0),
      (0, 1, 1, 0, -1, 0, 0, 0, 0), (0, 1, 0, 0, 1, 0, 0, 1, 0), (1, 0, 0, 0, -1, 0, 1, 0, 0))
_PLAIN = {0: 2, 1: 1, 2: 4, 12: 0, 13: 3}
_SUMS = (("n7", "p8", "+p11"), ("n6", "p7", "-p6"), ("n5", "p4", "+n6"), ("n4", "p0", "-n7"),
         ("n3", "p14", "+n5"), ("n2", "p9", "+n4", "+n3"), ("n1", "p5", "+n2"),
         (0, "n1", "-n4", "+p1", "+p6"), (1, "p12", "+n7", "+p3", "-n6"), (2, "n1", "-p3"),
         (3, "p2", "-n3"), (4, "p13", "+n5", "-p11"), (5, "p10", "-n2"))


def _left_forms(a):
    a0, a1, a2, a3, a4, a5 = a
    t0 = a3 - a5
    t1 = a4 - a5
    t2 = a2 - t0
    t3 = a0 - t2
    t4 = a1 + t3
    t5 = t4 - t0
    t6 = a2 - t1
    t7 = a2 + a5
    t8 = t1 + t5
    t9 = t8 - a0
    return (a2, a1, a4, t3, t8, t9, t4, t5, t2, t6, t7, t0, a0, a3, t1)


def _right_forms(block, put):
    for r, coefs in enumerate(_V):
        terms = sorted(((cf, j) for j, cf in enumerate(coefs) if cf), key=lambda t: -t[0])
        acc = block(*divmod(terms[0][1], 3))
        if terms[0][0] < 0:
            acc = -acc
        for cf, j in terms[1:]:
            acc = acc + block(*divmod(j, 3)) if cf > 0 else acc - block(*divmod(j, 3))
        put(r, acc.astype(jnp.bfloat16))


class _Combiner:
    def __init__(self, emit):
        self.emit, self.val = emit, {}
        self.todo = [[name, None, ["+" + terms[0], *terms[1:]]] for name, *terms in _SUMS]

    def put(self, r, v):
        self.val["p%d" % r] = v
        for item in self.todo:
            name, acc, terms = item
            ready = [t for t in terms if t[1:] in self.val]
            if acc is None:
                first = [t for t in ready if t[0] == "+"][:1]
                if not first or len(ready) < 2:
                    continue
                acc = self.val[first[0][1:]]
                ready.remove(first[0])
                terms.remove(first[0])
            for t in ready:
                acc = acc + self.val[t[1:]] if t[0] == "+" else acc - self.val[t[1:]]
                terms.remove(t)
            item[1] = acc
            if ready and not terms:
                if isinstance(name, str):
                    self.val[name] = acc
                else:
                    self.emit(name, acc)


def _combine(p):
    val = {"p%d" % r: v for r, v in enumerate(p)}
    for name, first, *rest in _SUMS:
        acc = val[first]
        for t in rest:
            acc = acc + val[t[1:]] if t[0] == "+" else acc - val[t[1:]]
        val[name] = acc
    return [val[q] for q in range(6)]


def _interleave(main, *side, spread):
    items = [((j + 1.0) / len(main), 1, j, f) for j, f in enumerate(main)]
    for st, begin, end in side:
        items += [(begin + (end - begin) * (j + 1.0) / len(st) - 1e-9, 0, j, f) for j, f in enumerate(st)]
    items.sort(key=lambda t: t[:3])
    pending = []
    for _, is_main, _, f in items:
        if is_main:
            f(pending[:spread])
            pending = pending[spread:]
        else:
            pending = pending + list(f())


def _body(x_hbm, dw_ref, w1_hbm, w2_ref, g_ref, b_ref, o_hbm, h_hbm,
          xbuf, hbuf, ssq, zero_ref, xsem, hsem, osem, x2sem, *, n, c):
    f32, bf16, i32 = jnp.float32, jnp.bfloat16, jnp.int32
    tm = 2 * R
    nb = n // tm
    nu = nb - NCACHE
    hc = 4 * c
    kb, nbk = c // 3, hc // 3
    rw = R // 2
    nt = R // 16

    def pack(lo, hi):
        return pltpu.bitcast(pltpu.pack_elementwise([lo, hi], packed_dtype=bf16), i32)

    def unpack(w):
        return [pltpu.unpack_elementwise(w, index=k, packed_dtype=bf16, unpacked_dtype=f32) for k in range(2)]

    def x_rows(i):
        return x_hbm.at[pl.ds(pl.multiple_of(i * tm, tm), tm)]

    def x_copy(i):
        return pltpu.make_async_copy(x_rows(i), xbuf.at[i % NXB], xsem.at[i % NXB])

    def h_rows(u):
        return h_hbm.at[pl.ds(pl.multiple_of(u * R, R), R)]

    def h_out_copy(u, s):
        return pltpu.make_async_copy(hbuf.at[s], h_rows(u), hsem.at[s])

    def h_in_copy(u, s):
        return pltpu.make_async_copy(h_rows(u), hbuf.at[s], hsem.at[s])

    def placement(i, state):
        rem, before, stage = state
        cached = rem + NCACHE >= nb
        return cached, i - before, stage, jnp.where(cached, NHB + before, stage)

    def advance(state):
        rem, before, stage = state
        cached = rem + NCACHE >= nb
        nxt = jnp.where(stage == NHB - 1, 0, stage + 1)
        return (jnp.where(cached, rem + NCACHE - nb, rem + NCACHE), before + cached.astype(i32),
                jnp.where(cached, stage, nxt))

    def retreat(state):
        rem, before, stage = state
        cached = rem < NCACHE
        prv = jnp.where(stage == 0, NHB - 1, stage - 1)
        return (jnp.where(cached, rem - NCACHE + nb, rem - NCACHE), before - cached.astype(i32),
                jnp.where(cached, stage, prv))

    def products(lhs, rhs, put, order):
        never = (jax.lax.broadcasted_iota(i32, (8, 128), 0) + zero_ref[0]) < 0
        rows = []

        def piece(r, t):
            def run(ties):
                v = lhs(r, t)
                if ties:
                    tie = functools.reduce(jnp.bitwise_or, [pltpu.bitcast(z, i32) for z in ties])
                    head = jnp.where(never, tie, v[:, :128])
                    v = head if v.shape[1] == 128 else jnp.concatenate([head, v[:, 128:]], axis=1)
                rows.append(v)
                if t == nt - 1:
                    a = pltpu.bitcast(jnp.concatenate(rows, axis=0), bf16)
                    rows.clear()
                    put(r, jnp.dot(a, rhs(r), preferred_element_type=f32))
            return run
        return [piece(r, t) for r in order for t in range(nt)]

    def prepare_w1(w1c, w1_ref):
        cp = pltpu.make_async_copy(w1_hbm, w1_ref, osem.at[0])
        cp.start()
        cp.wait()

        def put(r, v):
            w1c[pl.ds(r * kb, kb), :] = v
        _right_forms(lambda j, k: w1_ref[j * kb:(j + 1) * kb, k * nbk:(k + 1) * nbk].astype(f32), put)

    def pass1(w1c, fa, fb, pa, pb):
        dw = dw_ref[...].astype(f32)

        def layer_norm(xv):
            o = xv * dw
            d = o - jnp.sum(o, axis=-1, keepdims=True) * (1.0 / c)
            v = jnp.sum(d * d, axis=-1, keepdims=True)
            return d * jax.lax.rsqrt(v * (1.0 / (c * _A * _A)) + 1e-5 / (_A * _A))

        def normalize(i, fs):
            xs, f = i % NXB, fs.bitcast(bf16)

            def piece(t):
                def run():
                    a = []
                    for half in range(2):
                        w = pltpu.bitcast(xbuf[xs, pl.ds(half * R + 16 * t, 16), :], i32)
                        ln = layer_norm(jnp.concatenate(unpack(w), axis=0))
                        a += [ln[:, j * kb:(j + 1) * kb] for j in range(3)]
                    for r, form in enumerate(_left_forms(a)):
                        f[pl.ds(16 * t, 16), pl.ds(r * kb, kb)] = form.astype(bf16)
                    return []
                return run
            return [piece(t) for t in range(nt)]

        def multiply(fs, ps):
            def put(r, v):
                ps[:, pl.ds(r * nbk, nbk)] = v
            return products(lambda r, t: fs[pl.ds(8 * t, 8), pl.ds(r * kb, kb)],
                            lambda r: w1c[pl.ds(r * kb, kb), :], put, range(15))

        def activate(hs, ps):
            acc = {}

            def piece(j, t):
                def run():
                    cs = _combine([ps[pl.ds(16 * t, 16), pl.ds(r * nbk + 128 * j, 128)] for r in range(15)])
                    for k in range(3):
                        cols = pl.ds(k * nbk + 128 * j, 128)
                        if t == 0:
                            acc[k] = ssq[:, cols]
                        for half in range(2):
                            y = cs[3 * half + k]
                            hh = y * (1.0 + jnp.tanh(y * (y * y + _KK)))
                            hbuf[hs, pl.ds(half * rw + 8 * t, 8), cols] = pack(hh[:8], hh[8:])
                            sq = hh * hh
                            acc[k] = acc[k] + (sq[:8] + sq[8:])
                        if t == nt - 1:
                            ssq[:, cols] = acc[k]
                    return [acc[k] for k in range(3)]
                return run
            return [piece(j, t) for j in range(nbk // 128) for t in range(nt)]

        x_copy(0).wait()
        x_copy(1).wait()
        for f in normalize(0, fa):
            f()
        _interleave(multiply(fa, pa), (normalize(1, fb),) + W11, spread=1)
        for j in range(2):
            x_copy(NXB + j).start()

        def step(i, state, f0, f1, p0, p1):
            cached, u, stage, slot = placement(i, state)

            @pl.when(i + 2 < nb)
            def _():
                x_copy(i + 2).wait()

            @pl.when(jnp.logical_and(jnp.logical_not(cached), u >= NHB))
            def _():
                h_out_copy(u - NHB, stage).wait()

            _interleave(multiply(f1, p1), (normalize(i + 2, f0),) + W11, (activate(slot, p0),) + W13, spread=1)

            @pl.when(i + NXB + 2 < nb)
            def _():
                x_copy(i + NXB + 2).start()

            @pl.when(jnp.logical_and(jnp.logical_not(cached), u < nu - NHB))
            def _():
                h_out_copy(u, stage).start()

            return advance(state)

        def two_steps(k, state):
            state = step(2 * k, state, fa, fb, pa, pb)
            return step(2 * k + 1, state, fb, fa, pb, pa)

        jax.lax.fori_loop(0, nb // 2, two_steps, (jnp.int32(0),) * 3)

    def phase1(w1c):
        w1c = w1c.bitcast(bf16)
        pl.run_scoped(functools.partial(prepare_w1, w1c), pltpu.VMEM((c, hc), bf16))
        pl.run_scoped(functools.partial(pass1, w1c),
                      pltpu.VMEM((rw, 15 * kb), i32), pltpu.VMEM((rw, 15 * kb), i32),
                      pltpu.VMEM((R, 15 * nbk), f32), pltpu.VMEM((R, 15 * nbk), f32))

    def pass2(w2c, obuf, xres):
        w2c = w2c.bitcast(bf16)

        def o_copy(b):
            rows = pl.ds(pl.multiple_of(b * (OB * tm), OB * tm), OB * tm)
            return pltpu.make_async_copy(obuf.at[b % 2], o_hbm.at[rows], osem.at[b % 2])

        def res_copy(i):
            return pltpu.make_async_copy(x_rows(i), xres.at[i % NX2], x2sem.at[i % NX2])

        for i in range(nb - 1, nb - 1 - NX2, -1):
            if i >= nb - NXB:
                pltpu.make_async_copy(xbuf.at[i % NXB], xres.at[i % NX2], x2sem.at[i % NX2]).start()
            else:
                res_copy(i).start()

        gx = jnp.sqrt(jnp.sum(ssq[...], axis=0, keepdims=True) * (_HS * _HS) + 1e-6)
        nx = gx / (jnp.mean(gx, axis=-1, keepdims=True) + 1e-6)
        scale = (g_ref[...].astype(f32) * nx + 1.0) * _HS
        scale = jnp.transpose(jnp.broadcast_to(scale, (128, hc)))

        def put(r, v):
            w2c[:, pl.ds(r * kb, kb)] = v
        _right_forms(lambda j, k: w2_ref[j * nbk:(j + 1) * nbk, k * kb:(k + 1) * kb].astype(f32)
                     * scale[j * nbk:(j + 1) * nbk], put)
        bias = jnp.dot(jnp.broadcast_to(b_ref[...], (16, hc)), w2_ref[...], preferred_element_type=f32)[0:1]

        def work(i, hs):
            ob = obuf.at[(i // OB) % 2, pl.ds(pl.multiple_of((i % OB) * tm, tm), tm)]
            xs = i % NX2
            forms = {}

            def h_words(q, t, off, width):
                return hbuf[hs, pl.ds((q // 3) * rw + 8 * t, 8), pl.ds((q % 3) * nbk + off, width)]

            def form_piece(t, j):
                def run():
                    a = [unpack(h_words(q, t, 128 * j, 128)) for q in range(6)]
                    lo, hi = [_left_forms([v[e] for v in a]) for e in range(2)]
                    for r in range(15):
                        if r not in _PLAIN:
                            forms[r, t, j] = pack(lo[r], hi[r])
                    return [forms[r, t, j] for r in TIE2]
                return run

            def lhs(r, t):
                if r in _PLAIN:
                    return h_words(_PLAIN[r], t, 0, nbk)
                return jnp.concatenate([forms[r, t, j] for j in range(nbk // 128)], axis=1)

            def emit(q, y):
                half, k = divmod(q, 3)
                rows, cols = pl.ds(half * R, R), pl.ds(k * kb, kb)
                ob[rows, cols] = (y + (bias[:, k * kb:(k + 1) * kb] + xres[xs, rows, cols].astype(f32))).astype(bf16)

            _interleave(products(lhs, lambda r: w2c[:, pl.ds(r * kb, kb)], _Combiner(emit).put, ORDER2),
                        ([form_piece(t, j) for t in range(nt) for j in range(nbk // 128)],) + W21, spread=1000)

        def step(k, state):
            i = nb - 1 - k
            cached, u, stage, slot = placement(i, state)

            @pl.when(jnp.logical_and(jnp.logical_not(cached), u < nu - NHB))
            def _():
                h_in_copy(u, stage).wait()

            res_copy(i).wait()

            @pl.when(jnp.logical_and(i % OB == OB - 1, i // OB + 2 < nb // OB))
            def _():
                o_copy(i // OB + 2).wait()

            work(i, slot)

            @pl.when(i % OB == 0)
            def _():
                o_copy(i // OB).start()

            @pl.when(jnp.logical_and(jnp.logical_not(cached), u >= NHB))
            def _():
                h_in_copy(u - NHB, stage).start()

            @pl.when(i >= NX2)
            def _():
                res_copy(i - NX2).start()

            return retreat(state)

        end = (jnp.int32(0), jnp.int32(NCACHE), jnp.int32(nu % NHB))
        jax.lax.fori_loop(0, nb, step, retreat(end))
        o_copy(1).wait()
        o_copy(0).wait()

    zero_ref[0] = 0
    ssq[...] = jnp.zeros_like(ssq)
    if PH1:
        for j in range(NXB):
            x_copy(j).start()
        pl.run_scoped(phase1, pltpu.VMEM((15 * kb // 2, nbk), i32))
    if PH2:
        pl.run_scoped(pass2, pltpu.VMEM((nbk // 2, 15 * kb), i32), pltpu.VMEM((2, OB * tm, c), bf16),
                      pltpu.VMEM((NX2, tm, c), bf16))


@jax.jit
def pallas_standalone__modern_conv_block_slak__vision_kernel(x, dw, w1, w2, grn_g, grn_b):
    bsz, hh, ww, c = x.shape
    assert bsz == 1 and dw.shape[:2] == (1, 1)
    n = hh * ww
    nb = n // (2 * R)
    vmem = pl.BlockSpec(memory_space=pltpu.VMEM)
    hbm = pl.BlockSpec(memory_space=pl.ANY)
    out, _ = pl.pallas_call(
        functools.partial(_body, n=n, c=c),
        in_specs=[hbm, vmem, hbm, vmem, vmem, vmem],
        out_specs=[hbm, hbm],
        out_shape=[jax.ShapeDtypeStruct((n, c), x.dtype),
                   jax.ShapeDtypeStruct(((nb - NCACHE - NHB) * R, 4 * c), jnp.int32)],
        scratch_shapes=[
            pltpu.VMEM((NXB, 2 * R, c), x.dtype),
            pltpu.VMEM((NHB + NCACHE, R, 4 * c), jnp.int32),
            pltpu.VMEM((8, 4 * c), jnp.float32),
            pltpu.SMEM((1,), jnp.int32),
            pltpu.SemaphoreType.DMA((NXB,)),
            pltpu.SemaphoreType.DMA((NHB,)),
            pltpu.SemaphoreType.DMA((2,)),
            pltpu.SemaphoreType.DMA((NX2,)),
        ],
        compiler_params=pltpu.CompilerParams(vmem_limit_bytes=VMEM_LIMIT, flags=FLAGS),
    )(x.reshape(n, c), dw.reshape(1, c), w1, w2, grn_g.reshape(1, 4 * c), grn_b.reshape(1, 4 * c))
    return out.reshape(x.shape)
```

```python
import functools
import math

import jax
import jax.numpy as jnp
import jax.experimental.pallas as pl
import jax.experimental.pallas.tpu as pltpu

R = 256
NCACHE = 69
NHB = 6
NXB = 4
NX2 = 8
OB = 4
VMEM_LIMIT = 128 * 1024 * 1024
W11 = (0.1, 1.0)
W13 = (0.02, 1.0)
W21 = (0.01, 0.33)
TIE2 = (5, 9, 10)
ORDER2 = (0, 1, 2, 12, 13, 11, 8, 6, 7, 4, 14, 9, 3, 5, 10)
FLAGS = {"XLA_TPU_EVENLY_DISTRIBUTE_CRITICAL_NODES": True}
F2 = dict(FLAGS, XLA_TPU_RESCHEDULE_DMA_DONES=True)
MARGIN = -2
CELLS = 15
PH1 = True
PH2 = True

_C1 = math.sqrt(2.0 / math.pi)
_A = (_C1 * 0.044715) ** (1.0 / 3.0)
_KK = _C1 / _A
_HS = 0.5 / _A

_V = ((-1, 0, 0, 0, 1, 0, -1, 1, 1), (-1, 0, 0, 1, 0, -1, 0, 0, 0), (1, 0, 0, 1, 0, 0, 1, 0, 0),
      (0, 0, -1, 0, 0, 0, 0, 0, 0), (0, 0, 0, 0, 1, 0, 0, 0, 0), (0, 0, 0, 0, 0, 1, 0, 0, 0),
      (1, 0, 0, 0, 0, 0, 0, 0, 0), (1, 0, 0, 0, -1, 0, 0, 0, 0), (0, 0, -1, 0, 1, 0, 0, 1, 0),
      (1, 0, 0, 0, 0, 1, 1, 0, 0), (0, 0, 1, 0, 0, 1, 0, 0, 1), (-1, 0, 0, 0, 1, 0, 0, 1, 0),
      (0, 1, 1, 0, -1, 0, 0, 0, 0), (0, 1, 0, 0, 1, 0, 0, 1, 0), (1, 0, 0, 0, -1, 0, 1, 0, 0))
_PLAIN = {0: 2, 1: 1, 2: 4, 12: 0, 13: 3}
_SUMS = (("n7", "p8", "+p11"), ("n6", "p7", "-p6"), ("n5", "p4", "+n6"), ("n4", "p0", "-n7"),
         ("n3", "p14", "+n5"), ("n2", "p9", "+n4", "+n3"), ("n1", "p5", "+n2"),
         (0, "n1", "-n4", "+p1", "+p6"), (1, "p12", "+n7", "+p3", "-n6"), (2, "n1", "-p3"),
         (3, "p2", "-n3"), (4, "p13", "+n5", "-p11"), (5, "p10", "-n2"))


def _left_forms(a):
    a0, a1, a2, a3, a4, a5 = a
    t0 = a3 - a5
    t1 = a4 - a5
    t2 = a2 - t0
    t3 = a0 - t2
    t4 = a1 + t3
    t5 = t4 - t0
    t6 = a2 - t1
    t7 = a2 + a5
    t8 = t1 + t5
    t9 = t8 - a0
    return (a2, a1, a4, t3, t8, t9, t4, t5, t2, t6, t7, t0, a0, a3, t1)


def _right_forms(block, put):
    for r, coefs in enumerate(_V):
        terms = sorted(((cf, j) for j, cf in enumerate(coefs) if cf), key=lambda t: -t[0])
        acc = block(*divmod(terms[0][1], 3))
        if terms[0][0] < 0:
            acc = -acc
        for cf, j in terms[1:]:
            acc = acc + block(*divmod(j, 3)) if cf > 0 else acc - block(*divmod(j, 3))
        put(r, acc.astype(jnp.bfloat16))


class _Combiner:
    def __init__(self, emit):
        self.emit, self.val = emit, {}
        self.todo = [[name, None, ["+" + terms[0], *terms[1:]]] for name, *terms in _SUMS]

    def put(self, r, v):
        self.val["p%d" % r] = v
        for item in self.todo:
            name, acc, terms = item
            ready = [t for t in terms if t[1:] in self.val]
            if acc is None:
                first = [t for t in ready if t[0] == "+"][:1]
                if not first or len(ready) < 2:
                    continue
                acc = self.val[first[0][1:]]
                ready.remove(first[0])
                terms.remove(first[0])
            for t in ready:
                acc = acc + self.val[t[1:]] if t[0] == "+" else acc - self.val[t[1:]]
                terms.remove(t)
            item[1] = acc
            if ready and not terms:
                if isinstance(name, str):
                    self.val[name] = acc
                else:
                    self.emit(name, acc)


def _combine(p):
    val = {"p%d" % r: v for r, v in enumerate(p)}
    for name, first, *rest in _SUMS:
        acc = val[first]
        for t in rest:
            acc = acc + val[t[1:]] if t[0] == "+" else acc - val[t[1:]]
        val[name] = acc
    return [val[q] for q in range(6)]


def _interleave(main, *side, spread):
    items = [((j + 1.0) / len(main), 1, j, f) for j, f in enumerate(main)]
    for st, begin, end in side:
        items += [(begin + (end - begin) * (j + 1.0) / len(st) - 1e-9, 0, j, f) for j, f in enumerate(st)]
    items.sort(key=lambda t: t[:3])
    pending = []
    for _, is_main, _, f in items:
        if is_main:
            f(pending[:spread])
            pending = pending[spread:]
        else:
            pending = pending + list(f())


def _product_cells(units, margin):
    keys = [(r, u) for r in range(15) for u in range(units)]
    even = {key: n for n, key in enumerate(keys)}
    odd, taken, size = {}, set(), len(keys)
    for r, u in keys:
        first = -(-15 * (u + 1 + margin) // units)
        last = min(r * units // 15 - 1 - margin, units - 1)
        free = [(q, w) for q in range(first, 15) for w in range(last, -1, -1) if (q, w) not in taken]
        if free:
            taken.add(free[0])
            odd[r, u] = even[free[0]]
        else:
            odd[r, u] = size
            size += 1
    return even, odd, size


def _when(cond, action):
    return lambda: pl.when(cond)(action)


def _body(x_hbm, dw_ref, w1_hbm, w2_ref, g_ref, b_ref, o_hbm, h_hbm,
          xbuf, hbuf, ssq, zero_ref, xsem, hsem, osem, x2sem, *, n, c):
    f32, bf16, i32 = jnp.float32, jnp.bfloat16, jnp.int32
    tm = 2 * R
    nb = n // tm
    nu = nb - NCACHE
    hc = 4 * c
    kb, nbk = c // 3, hc // 3
    rw = R // 2
    nt = R // 16

    def pack(lo, hi):
        return pltpu.bitcast(pltpu.pack_elementwise([lo, hi], packed_dtype=bf16), i32)

    def unpack(w):
        return [pltpu.unpack_elementwise(w, index=k, packed_dtype=bf16, unpacked_dtype=f32) for k in range(2)]

    def x_rows(i):
        return x_hbm.at[pl.ds(pl.multiple_of(i * tm, tm), tm)]

    def x_copy(i):
        return pltpu.make_async_copy(x_rows(i), xbuf.at[i % NXB], xsem.at[i % NXB])

    def h_rows(u):
        return h_hbm.at[pl.ds(pl.multiple_of(u * R, R), R)]

    def h_out_copy(u, s):
        return pltpu.make_async_copy(hbuf.at[s], h_rows(u), hsem.at[s])

    def h_in_copy(u, s):
        return pltpu.make_async_copy(h_rows(u), hbuf.at[s], hsem.at[s])

    def placement(i, state):
        rem, before, stage = state
        cached = rem + NCACHE >= nb
        return cached, i - before, stage, jnp.where(cached, NHB + before, stage)

    def advance(state):
        rem, before, stage = state
        cached = rem + NCACHE >= nb
        nxt = jnp.where(stage == NHB - 1, 0, stage + 1)
        return (jnp.where(cached, rem + NCACHE - nb, rem + NCACHE), before + cached.astype(i32),
                jnp.where(cached, stage, nxt))

    def retreat(state):
        rem, before, stage = state
        cached = rem < NCACHE
        prv = jnp.where(stage == 0, NHB - 1, stage - 1)
        return (jnp.where(cached, rem - NCACHE + nb, rem - NCACHE), before - cached.astype(i32),
                jnp.where(cached, stage, prv))

    def products(lhs, rhs, put, order):
        never = (jax.lax.broadcasted_iota(i32, (8, 128), 0) + zero_ref[0]) < 0
        rows = []

        def piece(r, t):
            def run(ties):
                v = lhs(r, t)
                if ties:
                    tie = functools.reduce(jnp.bitwise_or, [pltpu.bitcast(z, i32) for z in ties])
                    head = jnp.where(never, tie, v[:, :128])
                    v = head if v.shape[1] == 128 else jnp.concatenate([head, v[:, 128:]], axis=1)
                rows.append(v)
                if t == nt - 1:
                    a = pltpu.bitcast(jnp.concatenate(rows, axis=0), bf16)
                    rows.clear()
                    put(r, jnp.dot(a, rhs(r), preferred_element_type=f32))
            return run
        return [piece(r, t) for r in order for t in range(nt)]

    def layer_norm(xv):
        o = xv * dw_ref[...].astype(f32)
        d = o - jnp.sum(o, axis=-1, keepdims=True) * (1.0 / c)
        v = jnp.sum(d * d, axis=-1, keepdims=True)
        return d * jax.lax.rsqrt(v * (1.0 / (c * _A * _A)) + 1e-5 / (_A * _A))

    def normalize(i, fs):
        xs, f = i % NXB, fs.bitcast(bf16)

        def piece(t):
            def run():
                a = []
                for half in range(2):
                    w = pltpu.bitcast(xbuf[xs, pl.ds(half * R + 16 * t, 16), :], i32)
                    ln = layer_norm(jnp.concatenate(unpack(w), axis=0))
                    a += [ln[:, j * kb:(j + 1) * kb] for j in range(3)]
                for r, form in enumerate(_left_forms(a)):
                    f[pl.ds(16 * t, 16), pl.ds(r * kb, kb)] = form.astype(bf16)
                return []
            return run
        return [piece(t) for t in range(nt)]

    def prepare(w1c, fa, w1_ref):
        cp = pltpu.make_async_copy(w1_hbm, w1_ref, osem.at[0])
        cp.start()
        x_copy(0).wait()
        for f in normalize(0, fa):
            f()
        cp.wait()

        def put(r, v):
            w1c[pl.ds(r * kb, kb), :] = v
        _right_forms(lambda j, k: w1_ref[j * kb:(j + 1) * kb, k * nbk:(k + 1) * nbk].astype(f32), put)

    even, odd, ncell = _product_cells(nt * nbk // 128, MARGIN)

    def pass1(w1c, fa, fb, pool):
        unread = set()

        def cell(where, r, j, t, write):
            idx = where[r, j * nt + t]
            assert (idx in unread) != write, "product cell reused before it was read"
            unread.add(idx) if write else unread.remove(idx)
            row, col = divmod(idx, CELLS)
            return pool.at[pl.ds(16 * row, 16), pl.ds(128 * col, 128)]

        def multiply(fs, ps):
            def put(r, v):
                for t in range(nt):
                    for j in range(nbk // 128):
                        cell(ps, r, j, t, True)[...] = v[16 * t:16 * t + 16, 128 * j:128 * j + 128]
            return products(lambda r, t: fs[pl.ds(8 * t, 8), pl.ds(r * kb, kb)],
                            lambda r: w1c[pl.ds(r * kb, kb), :], put, range(15))

        def activate(hs, ps):
            acc = {}

            def piece(j, t):
                def run():
                    cs = _combine([cell(ps, r, j, t, False)[...] for r in range(15)])
                    for k in range(3):
                        cols = pl.ds(k * nbk + 128 * j, 128)
                        if t == 0:
                            acc[k] = ssq[:, cols]
                        for half in range(2):
                            y = cs[3 * half + k]
                            hh = y * (1.0 + jnp.tanh(y * (y * y + _KK)))
                            hbuf[hs, pl.ds(half * rw + 8 * t, 8), cols] = pack(hh[:8], hh[8:])
                            sq = hh * hh
                            acc[k] = acc[k] + (sq[:8] + sq[8:])
                        if t == nt - 1:
                            ssq[:, cols] = acc[k]
                    return [acc[k] for k in range(3)]
                return run
            return [piece(j, t) for j in range(nbk // 128) for t in range(nt)]

        pa, pb = even, odd
        x_copy(1).wait()
        _interleave(multiply(fa, pa), (normalize(1, fb),) + W11, spread=1)
        for j in range(2):
            x_copy(NXB + j).start()

        def input_waits(i, state):
            cached, u, stage, slot = placement(i, state)
            return slot, [_when(i + 2 < nb, x_copy(jnp.minimum(i + 2, nb - 1)).wait),
                          _when((i < nb) & jnp.logical_not(cached) & (u >= NHB), h_out_copy(0, stage).wait)]

        def step(i, carry, f0, f1, p0, p1):
            state, slot = carry
            cached, u, stage, _ = placement(i, state)
            state = advance(state)
            next_slot, waits = input_waits(i + 1, state)
            starts = [_when(i + NXB + 2 < nb, x_copy(jnp.minimum(i + NXB + 2, nb - 1)).start),
                      _when(jnp.logical_not(cached) & (u < nu - NHB),
                            h_out_copy(jnp.minimum(u, nu - NHB - 1), stage).start)]
            _interleave(multiply(f1, p1), (normalize(i + 2, f0),) + W11, (activate(slot, p0),) + W13, spread=1)
            for action in starts + waits:
                action()
            return state, next_slot

        def two_steps(k, carry):
            carry = step(2 * k, carry, fa, fb, pa, pb)
            return step(2 * k + 1, carry, fb, fa, pb, pa)

        start = (jnp.int32(0),) * 3
        slot, waits = input_waits(jnp.int32(0), start)
        for action in waits:
            action()
        jax.lax.fori_loop(0, nb // 2, two_steps, (start, slot))

    def phase1(w1c, fa, fb):
        w1c = w1c.bitcast(bf16)
        pl.run_scoped(functools.partial(prepare, w1c, fa), pltpu.VMEM((c, hc), bf16))
        pl.run_scoped(functools.partial(pass1, w1c, fa, fb),
                      pltpu.VMEM((16 * pl.cdiv(ncell, CELLS), 128 * CELLS), f32))

    def pass2(w2c, obuf, xres):
        w2c = w2c.bitcast(bf16)

        ng = nb // OB

        def o_copy(b):
            rows = pl.ds(pl.multiple_of(b * (OB * tm), OB * tm), OB * tm)
            return pltpu.make_async_copy(obuf.at[b % 2], o_hbm.at[rows], osem.at[b % 2])

        def res_copy(i):
            return pltpu.make_async_copy(x_rows(i), xres.at[i % NX2], x2sem.at[i % NX2])

        for i in range(nb - 1, nb - 1 - NX2, -1):
            if i >= nb - NXB:
                pltpu.make_async_copy(xbuf.at[i % NXB], xres.at[i % NX2], x2sem.at[i % NX2]).start()
            else:
                res_copy(i).start()

        gx = jnp.sqrt(jnp.sum(ssq[...], axis=0, keepdims=True) * (_HS * _HS) + 1e-6)
        nx = gx / (jnp.mean(gx, axis=-1, keepdims=True) + 1e-6)
        scale = (g_ref[...].astype(f32).reshape(1, hc) * nx + 1.0) * _HS
        scale = jnp.transpose(jnp.broadcast_to(scale, (128, hc)))

        def put(r, v):
            w2c[:, pl.ds(r * kb, kb)] = v
        _right_forms(lambda j, k: w2_ref[j * nbk:(j + 1) * nbk, k * kb:(k + 1) * kb].astype(f32)
                     * scale[j * nbk:(j + 1) * nbk], put)
        bias = jnp.dot(jnp.broadcast_to(b_ref[...].astype(f32).reshape(1, hc), (16, hc)).astype(bf16), w2_ref[...], preferred_element_type=f32)[0:1]

        def work(i, hs):
            ob = obuf.at[(i // OB) % 2, pl.ds(pl.multiple_of((i % OB) * tm, tm), tm)]
            xr = xres.at[i % NX2]
            forms = {}

            def h_words(q, t, off, width):
                return hbuf[hs, pl.ds((q // 3) * rw + 8 * t, 8), pl.ds((q % 3) * nbk + off, width)]

            def form_piece(t, j):
                def run():
                    a = [unpack(h_words(q, t, 128 * j, 128)) for q in range(6)]
                    lo, hi = [_left_forms([v[e] for v in a]) for e in range(2)]
                    for r in range(15):
                        if r not in _PLAIN:
                            forms[r, t, j] = pack(lo[r], hi[r])
                    return [forms[r, t, j] for r in TIE2]
                return run

            def lhs(r, t):
                if r in _PLAIN:
                    return h_words(_PLAIN[r], t, 0, nbk)
                return jnp.concatenate([forms[r, t, j] for j in range(nbk // 128)], axis=1)

            def emit(q, y):
                half, k = divmod(q, 3)
                rows, cols = pl.ds(half * R, R), pl.ds(k * kb, kb)
                ob[rows, cols] = (y + (bias[:, k * kb:(k + 1) * kb] + xr[rows, cols].astype(f32))).astype(bf16)

            _interleave(products(lhs, lambda r: w2c[:, pl.ds(r * kb, kb)], _Combiner(emit).put, ORDER2),
                        ([form_piece(t, j) for t in range(nt) for j in range(nbk // 128)],) + W21, spread=1000)

        def input_waits(i, state):
            cached, u, stage, slot = placement(i, state)
            group = jnp.maximum(i, 0) // OB
            first = (i >= 0) & (i % OB == OB - 1)
            return slot, [_when((i >= 0) & jnp.logical_not(cached) & (u < nu - NHB), h_in_copy(0, stage).wait),
                          _when(i >= 0, res_copy(jnp.maximum(i, 0)).wait),
                          _when(first & (group + 2 < ng), o_copy(jnp.minimum(group, ng - 3) + 2).wait)]

        def step(k, carry):
            i = nb - 1 - k
            state, slot = carry
            cached, u, stage, _ = placement(i, state)
            state = retreat(state)
            next_slot, waits = input_waits(i - 1, state)
            group, last = i // OB, i % OB == 0
            starts = [_when(jnp.logical_not(cached) & (u >= NHB), h_in_copy(jnp.maximum(u - NHB, 0), stage).start),
                      _when(last, o_copy(group).start),
                      _when(i >= NX2, res_copy(jnp.maximum(i - NX2, 0)).start)]
            work(i, slot)
            for action in starts + waits:
                action()
            return state, next_slot

        start = retreat((jnp.int32(0), jnp.int32(NCACHE), jnp.int32(nu % NHB)))
        slot, waits = input_waits(jnp.int32(nb - 1), start)
        for action in waits:
            action()
        jax.lax.fori_loop(0, nb, step, (start, slot))
        o_copy(1).wait()
        o_copy(0).wait()

    zero_ref[0] = 0
    ssq[...] = jnp.zeros_like(ssq)
    if PH1:
        for j in range(NXB):
            x_copy(j).start()
        pl.run_scoped(phase1, pltpu.VMEM((15 * kb // 2, nbk), i32),
                      pltpu.VMEM((rw, 15 * kb), i32), pltpu.VMEM((rw, 15 * kb), i32))
    if PH2:
        pl.run_scoped(pass2, pltpu.VMEM((nbk // 2, 15 * kb), i32), pltpu.VMEM((2, OB * tm, c), bf16),
                      pltpu.VMEM((NX2, tm, c), bf16))


@jax.jit
def pallas_standalone__modern_conv_block_slak__vision_kernel(x, dw, w1, w2, grn_g, grn_b):
    bsz, hh, ww, c = x.shape
    assert bsz == 1 and dw.shape[:2] == (1, 1)
    n = hh * ww
    nb = n // (2 * R)
    vmem = pl.BlockSpec(memory_space=pltpu.VMEM)
    hbm = pl.BlockSpec(memory_space=pl.ANY)
    out, _ = pl.pallas_call(
        functools.partial(_body, n=n, c=c),
        in_specs=[hbm, vmem, hbm, vmem, vmem, vmem],
        out_specs=[hbm, hbm],
        out_shape=[jax.ShapeDtypeStruct((n, c), x.dtype),
                   jax.ShapeDtypeStruct(((nb - NCACHE - NHB) * R, 4 * c), jnp.int32)],
        scratch_shapes=[
            pltpu.VMEM((NXB, 2 * R, c), x.dtype),
            pltpu.VMEM((NHB + NCACHE, R, 4 * c), jnp.int32),
            pltpu.VMEM((8, 4 * c), jnp.float32),
            pltpu.SMEM((1,), jnp.int32),
            pltpu.SemaphoreType.DMA((NXB,)),
            pltpu.SemaphoreType.DMA((NHB,)),
            pltpu.SemaphoreType.DMA((2,)),
            pltpu.SemaphoreType.DMA((NX2,)),
        ],
        compiler_params=pltpu.CompilerParams(vmem_limit_bytes=VMEM_LIMIT, flags=FLAGS),
    )(x.reshape(n, c), dw.reshape(1, c), w1, w2, grn_g, grn_b)
    return out.reshape(x.shape)
```

```python
import functools
import math

import jax
import jax.numpy as jnp
import jax.experimental.pallas as pl
import jax.experimental.pallas.tpu as pltpu

R = 256
NCACHE = 69
NHB = 6
NXB = 4
NX2 = 8
OB = 4
VMEM_LIMIT = 128 * 1024 * 1024
W11 = (0.1, 1.0)
W13 = (0.02, 1.0)
W21 = (0.01, 0.33)
TIE2 = (5, 9, 10)
ORDER2 = (0, 1, 2, 12, 13, 11, 8, 6, 7, 4, 14, 9, 3, 5, 10)
FLAGS = {"XLA_TPU_EVENLY_DISTRIBUTE_CRITICAL_NODES": True}
MARGIN = -2
CELLS = 15

_C1 = math.sqrt(2.0 / math.pi)
_A = (_C1 * 0.044715) ** (1.0 / 3.0)
_KK = _C1 / _A
_HS = 0.5 / _A

_V = ((-1, 0, 0, 0, 1, 0, -1, 1, 1), (-1, 0, 0, 1, 0, -1, 0, 0, 0), (1, 0, 0, 1, 0, 0, 1, 0, 0),
      (0, 0, -1, 0, 0, 0, 0, 0, 0), (0, 0, 0, 0, 1, 0, 0, 0, 0), (0, 0, 0, 0, 0, 1, 0, 0, 0),
      (1, 0, 0, 0, 0, 0, 0, 0, 0), (1, 0, 0, 0, -1, 0, 0, 0, 0), (0, 0, -1, 0, 1, 0, 0, 1, 0),
      (1, 0, 0, 0, 0, 1, 1, 0, 0), (0, 0, 1, 0, 0, 1, 0, 0, 1), (-1, 0, 0, 0, 1, 0, 0, 1, 0),
      (0, 1, 1, 0, -1, 0, 0, 0, 0), (0, 1, 0, 0, 1, 0, 0, 1, 0), (1, 0, 0, 0, -1, 0, 1, 0, 0))
_PLAIN = {0: 2, 1: 1, 2: 4, 12: 0, 13: 3}
_SUMS = (("n7", "p8", "+p11"), ("n6", "p7", "-p6"), ("n5", "p4", "+n6"), ("n4", "p0", "-n7"),
         ("n3", "p14", "+n5"), ("n2", "p9", "+n4", "+n3"), ("n1", "p5", "+n2"),
         (0, "n1", "-n4", "+p1", "+p6"), (1, "p12", "+n7", "+p3", "-n6"), (2, "n1", "-p3"),
         (3, "p2", "-n3"), (4, "p13", "+n5", "-p11"), (5, "p10", "-n2"))


def _left_forms(a):
    a0, a1, a2, a3, a4, a5 = a
    t0 = a3 - a5
    t1 = a4 - a5
    t2 = a2 - t0
    t3 = a0 - t2
    t4 = a1 + t3
    t5 = t4 - t0
    t6 = a2 - t1
    t7 = a2 + a5
    t8 = t1 + t5
    t9 = t8 - a0
    return (a2, a1, a4, t3, t8, t9, t4, t5, t2, t6, t7, t0, a0, a3, t1)


def _right_forms(block, put):
    for r, coefs in enumerate(_V):
        terms = sorted(((cf, j) for j, cf in enumerate(coefs) if cf), key=lambda t: -t[0])
        acc = block(*divmod(terms[0][1], 3))
        if terms[0][0] < 0:
            acc = -acc
        for cf, j in terms[1:]:
            acc = acc + block(*divmod(j, 3)) if cf > 0 else acc - block(*divmod(j, 3))
        put(r, acc.astype(jnp.bfloat16))


class _Combiner:
    def __init__(self, emit):
        self.emit, self.val = emit, {}
        self.todo = [[name, None, ["+" + terms[0], *terms[1:]]] for name, *terms in _SUMS]

    def put(self, r, v):
        self.val["p%d" % r] = v
        for item in self.todo:
            name, acc, terms = item
            ready = [t for t in terms if t[1:] in self.val]
            if acc is None:
                first = [t for t in ready if t[0] == "+"][:1]
                if not first or len(ready) < 2:
                    continue
                acc = self.val[first[0][1:]]
                ready.remove(first[0])
                terms.remove(first[0])
            for t in ready:
                acc = acc + self.val[t[1:]] if t[0] == "+" else acc - self.val[t[1:]]
                terms.remove(t)
            item[1] = acc
            if ready and not terms:
                if isinstance(name, str):
                    self.val[name] = acc
                else:
                    self.emit(name, acc)


def _combine(p):
    val = {"p%d" % r: v for r, v in enumerate(p)}
    for name, first, *rest in _SUMS:
        acc = val[first]
        for t in rest:
            acc = acc + val[t[1:]] if t[0] == "+" else acc - val[t[1:]]
        val[name] = acc
    return [val[q] for q in range(6)]


def _interleave(main, *side, spread):
    items = [((j + 1.0) / len(main), 1, j, f) for j, f in enumerate(main)]
    for st, begin, end in side:
        items += [(begin + (end - begin) * (j + 1.0) / len(st) - 1e-9, 0, j, f) for j, f in enumerate(st)]
    items.sort(key=lambda t: t[:3])
    pending = []
    for _, is_main, _, f in items:
        if is_main:
            f(pending[:spread])
            pending = pending[spread:]
        else:
            pending = pending + list(f())


def _product_cells(units, margin):
    keys = [(r, u) for r in range(15) for u in range(units)]
    even = {key: n for n, key in enumerate(keys)}
    odd, taken, size = {}, set(), len(keys)
    for r, u in keys:
        first = -(-15 * (u + 1 + margin) // units)
        last = min(r * units // 15 - 1 - margin, units - 1)
        free = [(q, w) for q in range(first, 15) for w in range(last, -1, -1) if (q, w) not in taken]
        if free:
            taken.add(free[0])
            odd[r, u] = even[free[0]]
        else:
            odd[r, u] = size
            size += 1
    return even, odd, size


def _when(cond, action):
    return lambda: pl.when(cond)(action)


def _body(x_hbm, dw_ref, w1_hbm, w2_ref, g_ref, b_ref, o_hbm, h_hbm,
          xbuf, hbuf, ssq, zero_ref, xsem, hsem, osem, x2sem, *, n, c):
    f32, bf16, i32 = jnp.float32, jnp.bfloat16, jnp.int32
    tm = 2 * R
    nb = n // tm
    nu = nb - NCACHE
    hc = 4 * c
    kb, nbk = c // 3, hc // 3
    rw = R // 2
    nt = R // 16

    def pack(lo, hi):
        return pltpu.bitcast(pltpu.pack_elementwise([lo, hi], packed_dtype=bf16), i32)

    def unpack(w):
        return [pltpu.unpack_elementwise(w, index=k, packed_dtype=bf16, unpacked_dtype=f32) for k in range(2)]

    def x_rows(i):
        return x_hbm.at[pl.ds(pl.multiple_of(i * tm, tm), tm)]

    def x_copy(i):
        return pltpu.make_async_copy(x_rows(i), xbuf.at[i % NXB], xsem.at[i % NXB])

    def h_rows(u):
        return h_hbm.at[pl.ds(pl.multiple_of(u * R, R), R)]

    def h_out_copy(u, s):
        return pltpu.make_async_copy(hbuf.at[s], h_rows(u), hsem.at[s])

    def h_in_copy(u, s):
        return pltpu.make_async_copy(h_rows(u), hbuf.at[s], hsem.at[s])

    def placement(i, state):
        rem, before, stage = state
        cached = rem + NCACHE >= nb
        return cached, i - before, stage, jnp.where(cached, NHB + before, stage)

    def advance(state):
        rem, before, stage = state
        cached = rem + NCACHE >= nb
        nxt = jnp.where(stage == NHB - 1, 0, stage + 1)
        return (jnp.where(cached, rem + NCACHE - nb, rem + NCACHE), before + cached.astype(i32),
                jnp.where(cached, stage, nxt))

    def retreat(state):
        rem, before, stage = state
        cached = rem < NCACHE
        prv = jnp.where(stage == 0, NHB - 1, stage - 1)
        return (jnp.where(cached, rem - NCACHE + nb, rem - NCACHE), before - cached.astype(i32),
                jnp.where(cached, stage, prv))

    def products(lhs, rhs, put, order):
        never = (jax.lax.broadcasted_iota(i32, (8, 128), 0) + zero_ref[0]) < 0
        rows = []

        def piece(r, t):
            def run(ties):
                v = lhs(r, t)
                if ties:
                    tie = functools.reduce(jnp.bitwise_or, [pltpu.bitcast(z, i32) for z in ties])
                    head = jnp.where(never, tie, v[:, :128])
                    v = head if v.shape[1] == 128 else jnp.concatenate([head, v[:, 128:]], axis=1)
                rows.append(v)
                if t == nt - 1:
                    a = pltpu.bitcast(jnp.concatenate(rows, axis=0), bf16)
                    rows.clear()
                    put(r, jnp.dot(a, rhs(r), preferred_element_type=f32))
            return run
        return [piece(r, t) for r in order for t in range(nt)]

    def layer_norm(xv):
        o = xv * dw_ref[...].astype(f32)
        d = o - jnp.sum(o, axis=-1, keepdims=True) * (1.0 / c)
        v = jnp.sum(d * d, axis=-1, keepdims=True)
        return d * jax.lax.rsqrt(v * (1.0 / (c * _A * _A)) + 1e-5 / (_A * _A))

    def normalize(i, fs):
        xs, f = i % NXB, fs.bitcast(bf16)

        def piece(t):
            def run():
                a = []
                for half in range(2):
                    w = pltpu.bitcast(xbuf[xs, pl.ds(half * R + 16 * t, 16), :], i32)
                    ln = layer_norm(jnp.concatenate(unpack(w), axis=0))
                    a += [ln[:, j * kb:(j + 1) * kb] for j in range(3)]
                for r, form in enumerate(_left_forms(a)):
                    f[pl.ds(16 * t, 16), pl.ds(r * kb, kb)] = form.astype(bf16)
                return []
            return run
        return [piece(t) for t in range(nt)]

    def prepare(w1c, fa, w1_ref):
        cp = pltpu.make_async_copy(w1_hbm, w1_ref, osem.at[0])
        cp.start()
        x_copy(0).wait()
        for f in normalize(0, fa):
            f()
        cp.wait()

        def put(r, v):
            w1c[pl.ds(r * kb, kb), :] = v
        _right_forms(lambda j, k: w1_ref[j * kb:(j + 1) * kb, k * nbk:(k + 1) * nbk].astype(f32), put)

    even, odd, ncell = _product_cells(nt * nbk // 128, MARGIN)

    def pass1(w1c, fa, fb, pool):
        unread = set()

        def cell(where, r, j, t, write):
            idx = where[r, j * nt + t]
            assert (idx in unread) != write, "product cell reused before it was read"
            unread.add(idx) if write else unread.remove(idx)
            row, col = divmod(idx, CELLS)
            return pool.at[pl.ds(16 * row, 16), pl.ds(128 * col, 128)]

        def multiply(fs, ps):
            def put(r, v):
                for t in range(nt):
                    for j in range(nbk // 128):
                        cell(ps, r, j, t, True)[...] = v[16 * t:16 * t + 16, 128 * j:128 * j + 128]
            return products(lambda r, t: fs[pl.ds(8 * t, 8), pl.ds(r * kb, kb)],
                            lambda r: w1c[pl.ds(r * kb, kb), :], put, range(15))

        def activate(hs, ps):
            acc = {}

            def piece(j, t):
                def run():
                    cs = _combine([cell(ps, r, j, t, False)[...] for r in range(15)])
                    for k in range(3):
                        cols = pl.ds(k * nbk + 128 * j, 128)
                        if t == 0:
                            acc[k] = ssq[:, cols]
                        for half in range(2):
                            y = cs[3 * half + k]
                            hh = y * (1.0 + jnp.tanh(y * (y * y + _KK)))
                            hbuf[hs, pl.ds(half * rw + 8 * t, 8), cols] = pack(hh[:8], hh[8:])
                            sq = hh * hh
                            acc[k] = acc[k] + (sq[:8] + sq[8:])
                        if t == nt - 1:
                            ssq[:, cols] = acc[k]
                    return [acc[k] for k in range(3)]
                return run
            return [piece(j, t) for j in range(nbk // 128) for t in range(nt)]

        pa, pb = even, odd
        x_copy(1).wait()
        _interleave(multiply(fa, pa), (normalize(1, fb),) + W11, spread=1)
        for j in range(2):
            x_copy(NXB + j).start()

        def input_waits(i, state):
            cached, u, stage, slot = placement(i, state)
            return slot, [_when(i + 2 < nb, x_copy(jnp.minimum(i + 2, nb - 1)).wait),
                          _when((i < nb) & jnp.logical_not(cached) & (u >= NHB), h_out_copy(0, stage).wait)]

        def step(i, carry, f0, f1, p0, p1):
            state, slot = carry
            cached, u, stage, _ = placement(i, state)
            state = advance(state)
            next_slot, waits = input_waits(i + 1, state)
            starts = [_when(i + NXB + 2 < nb, x_copy(jnp.minimum(i + NXB + 2, nb - 1)).start),
                      _when(jnp.logical_not(cached) & (u < nu - NHB),
                            h_out_copy(jnp.minimum(u, nu - NHB - 1), stage).start)]
            _interleave(multiply(f1, p1), (normalize(i + 2, f0),) + W11, (activate(slot, p0),) + W13, spread=1)
            for action in starts + waits:
                action()
            return state, next_slot

        def two_steps(k, carry):
            carry = step(2 * k, carry, fa, fb, pa, pb)
            return step(2 * k + 1, carry, fb, fa, pb, pa)

        start = (jnp.int32(0),) * 3
        slot, waits = input_waits(jnp.int32(0), start)
        for action in waits:
            action()
        jax.lax.fori_loop(0, nb // 2, two_steps, (start, slot))

    def phase1(w1c, fa, fb):
        w1c = w1c.bitcast(bf16)
        pl.run_scoped(functools.partial(prepare, w1c, fa), pltpu.VMEM((c, hc), bf16))
        pl.run_scoped(functools.partial(pass1, w1c, fa, fb),
                      pltpu.VMEM((16 * pl.cdiv(ncell, CELLS), 128 * CELLS), f32))

    def pass2(w2c, obuf, xres):
        w2c = w2c.bitcast(bf16)

        ng = nb // OB

        def o_copy(b):
            rows = pl.ds(pl.multiple_of(b * (OB * tm), OB * tm), OB * tm)
            return pltpu.make_async_copy(obuf.at[b % 2], o_hbm.at[rows], osem.at[b % 2])

        def res_copy(i):
            return pltpu.make_async_copy(x_rows(i), xres.at[i % NX2], x2sem.at[i % NX2])

        for i in range(nb - 1, nb - 1 - NX2, -1):
            if i >= nb - NXB:
                pltpu.make_async_copy(xbuf.at[i % NXB], xres.at[i % NX2], x2sem.at[i % NX2]).start()
            else:
                res_copy(i).start()

        gx = jnp.sqrt(jnp.sum(ssq[...], axis=0, keepdims=True) * (_HS * _HS) + 1e-6)
        nx = gx / (jnp.mean(gx, axis=-1, keepdims=True) + 1e-6)
        scale = (g_ref[...].astype(f32).reshape(1, hc) * nx + 1.0) * _HS
        scale = jnp.transpose(jnp.broadcast_to(scale, (128, hc)))

        def put(r, v):
            w2c[:, pl.ds(r * kb, kb)] = v
        _right_forms(lambda j, k: w2_ref[j * nbk:(j + 1) * nbk, k * kb:(k + 1) * kb].astype(f32)
                     * scale[j * nbk:(j + 1) * nbk], put)
        bias = jnp.dot(jnp.broadcast_to(b_ref[...].astype(f32).reshape(1, hc), (16, hc)).astype(bf16), w2_ref[...], preferred_element_type=f32)[0:1]

        def work(i, hs):
            ob = obuf.at[(i // OB) % 2, pl.ds(pl.multiple_of((i % OB) * tm, tm), tm)]
            xr = xres.at[i % NX2]
            forms = {}

            def h_words(q, t, off, width):
                return hbuf[hs, pl.ds((q // 3) * rw + 8 * t, 8), pl.ds((q % 3) * nbk + off, width)]

            def form_piece(t, j):
                def run():
                    a = [unpack(h_words(q, t, 128 * j, 128)) for q in range(6)]
                    lo, hi = [_left_forms([v[e] for v in a]) for e in range(2)]
                    for r in range(15):
                        if r not in _PLAIN:
                            forms[r, t, j] = pack(lo[r], hi[r])
                    return [forms[r, t, j] for r in TIE2]
                return run

            def lhs(r, t):
                if r in _PLAIN:
                    return h_words(_PLAIN[r], t, 0, nbk)
                return jnp.concatenate([forms[r, t, j] for j in range(nbk // 128)], axis=1)

            def emit(q, y):
                half, k = divmod(q, 3)
                rows, cols = pl.ds(half * R, R), pl.ds(k * kb, kb)
                ob[rows, cols] = (y + (bias[:, k * kb:(k + 1) * kb] + xr[rows, cols].astype(f32))).astype(bf16)

            _interleave(products(lhs, lambda r: w2c[:, pl.ds(r * kb, kb)], _Combiner(emit).put, ORDER2),
                        ([form_piece(t, j) for t in range(nt) for j in range(nbk // 128)],) + W21, spread=1000)

        def input_waits(i, state):
            cached, u, stage, slot = placement(i, state)
            group = jnp.maximum(i, 0) // OB
            first = (i >= 0) & (i % OB == OB - 1)
            return slot, [_when((i >= 0) & jnp.logical_not(cached) & (u < nu - NHB), h_in_copy(0, stage).wait),
                          _when(i >= 0, res_copy(jnp.maximum(i, 0)).wait),
                          _when(first & (group + 2 < ng), o_copy(jnp.minimum(group, ng - 3) + 2).wait)]

        def step(k, carry):
            i = nb - 1 - k
            state, slot = carry
            cached, u, stage, _ = placement(i, state)
            state = retreat(state)
            next_slot, waits = input_waits(i - 1, state)
            group, last = i // OB, i % OB == 0
            starts = [_when(jnp.logical_not(cached) & (u >= NHB), h_in_copy(jnp.clip(u - NHB, 0, nu - NHB - 1), stage).start),
                      _when(last, o_copy(group).start),
                      _when(i >= NX2, res_copy(jnp.maximum(i - NX2, 0)).start)]
            work(i, slot)
            for action in starts + waits:
                action()
            return state, next_slot

        start = retreat((jnp.int32(0), jnp.int32(NCACHE), jnp.int32(nu % NHB)))
        slot, waits = input_waits(jnp.int32(nb - 1), start)
        for action in waits:
            action()
        jax.lax.fori_loop(0, nb, step, (start, slot))
        o_copy(1).wait()
        o_copy(0).wait()

    zero_ref[0] = 0
    ssq[...] = jnp.zeros_like(ssq)
    for j in range(NXB):
        x_copy(j).start()
    pl.run_scoped(phase1, pltpu.VMEM((15 * kb // 2, nbk), i32),
                  pltpu.VMEM((rw, 15 * kb), i32), pltpu.VMEM((rw, 15 * kb), i32))
    pl.run_scoped(pass2, pltpu.VMEM((nbk // 2, 15 * kb), i32), pltpu.VMEM((2, OB * tm, c), bf16),
                  pltpu.VMEM((NX2, tm, c), bf16))


@jax.jit
def pallas_standalone__modern_conv_block_slak__vision_kernel(x, dw, w1, w2, grn_g, grn_b):
    bsz, hh, ww, c = x.shape
    assert bsz == 1 and dw.shape[:2] == (1, 1)
    n = hh * ww
    nb = n // (2 * R)
    vmem = pl.BlockSpec(memory_space=pltpu.VMEM)
    hbm = pl.BlockSpec(memory_space=pl.ANY)
    out, _ = pl.pallas_call(
        functools.partial(_body, n=n, c=c),
        in_specs=[hbm, vmem, hbm, vmem, vmem, vmem],
        out_specs=[hbm, hbm],
        out_shape=[jax.ShapeDtypeStruct((n, c), x.dtype),
                   jax.ShapeDtypeStruct(((nb - NCACHE - NHB) * R, 4 * c), jnp.int32)],
        scratch_shapes=[
            pltpu.VMEM((NXB, 2 * R, c), x.dtype),
            pltpu.VMEM((NHB + NCACHE, R, 4 * c), jnp.int32),
            pltpu.VMEM((8, 4 * c), jnp.float32),
            pltpu.SMEM((1,), jnp.int32),
            pltpu.SemaphoreType.DMA((NXB,)),
            pltpu.SemaphoreType.DMA((NHB,)),
            pltpu.SemaphoreType.DMA((2,)),
            pltpu.SemaphoreType.DMA((NX2,)),
        ],
        compiler_params=pltpu.CompilerParams(vmem_limit_bytes=VMEM_LIMIT, flags=FLAGS),
    )(x.reshape(n, c), dw.reshape(1, c), w1, w2, grn_g, grn_b)
    return out.reshape(x.shape)
```
